```python
import os as _os
_os.environ.setdefault("JAX_PLATFORMS", "cpu")
import jax
import jax.numpy as jnp

def _softmax(x, axis=-1):
    return jax.nn.softmax(x, axis=axis)
def _gelu(x):
    return jax.nn.gelu(x, approximate=True)
def _silu(x):
    return jax.nn.silu(x)
def _sigmoid(x):
    return jax.nn.sigmoid(x)
def _layernorm(x, axis=-1, eps=1e-5):
    m = jnp.mean(x, axis=axis, keepdims=True)
    v = jnp.var(x, axis=axis, keepdims=True)
    return (x - m) / jnp.sqrt(v + eps)
def _scatter_add(tgt, idx, src, axis=0):
    return tgt.at[idx].add(src)
def _segment_sum(src, seg, n):
    return jax.ops.segment_sum(src, seg, n)
class _Rng:
    def __init__(self, key):
        self._k = key
    def _next(self):
        self._k, sub = jax.random.split(self._k)
        return sub
    def normal(self, shape):
        return jax.random.normal(self._next(), shape, dtype=jnp.bfloat16)
    def randint(self, lo, hi, shape):
        return jax.random.randint(self._next(), shape, lo, hi, dtype=jnp.int32)
    def uniform(self, shape, lo=0.0, hi=1.0):
        return jax.random.uniform(self._next(), shape, jnp.bfloat16, lo, hi)
    def permutation(self, n):
        return jax.random.permutation(self._next(), n)


kernel_name = 'interleave_layers__sliding_local_dilated__sliding_local_dilated__prompt'

def setup_inputs():
    _rng = _Rng(jax.random.key(int.from_bytes(__import__("os").urandom(4), "little")))
    _w = (lambda a: (lambda t: t.astype(jnp.bfloat16) if jnp.issubdtype(t.dtype, jnp.floating) else t)(jnp.asarray(a)))
    def _A_setup():
        B, S, D = 1, 2048, 1024
        return {
            "x": _w((lambda *s: _rng.normal(s) * 0.05)(B, S, D)),
            "wqkv": _w((lambda *s: _rng.normal(s) * 0.05)(D, 3 * D)),
            "wo": _w((lambda *s: _rng.normal(s) * 0.05)(D, D)),
        }
    _A_in = _A_setup()

    def _B_setup():
        B, S, D = 1, 2048, 1024
        return {
            "x": _w((lambda *s: _rng.normal(s) * 0.05)(B, S, D)),
            "wqkv": _w((lambda *s: _rng.normal(s) * 0.05)(D, 3 * D)),
            "wo": _w((lambda *s: _rng.normal(s) * 0.05)(D, D)),
        }
    _B_in = _B_setup()

    return {
        "A_x": _A_in["x"],
        "A_wqkv": _A_in["wqkv"],
        "A_wo": _A_in["wo"],
        "B_x": _B_in["x"],
        "B_wqkv": _B_in["wqkv"],
        "B_wo": _B_in["wo"],
    }

def reference(A_x, A_wqkv, A_wo, B_x, B_wqkv, B_wo):
    def _A_ref(x, wqkv, wo):
        B, S, D = x.shape
        H = 32; Dh = D // H
        W, dil = 8, 2
        qkv = (lambda x, *d: x.transpose(*d))((x @ wqkv).reshape(B, S, 3, H, Dh), 2, 0, 3, 1, 4)
        q, k, v = qkv[0], qkv[1], qkv[2]
        scale = Dh ** -0.5
        pos = jnp.arange(S)
        off = jnp.arange(W) * dil
        idx = pos[:, None] - off[None, :]
        mask = idx >= 0
        idx_c = jnp.where(mask, idx, 0).reshape(-1)
        kg = k[:, :, idx_c, :].reshape(B, H, S, W, Dh)
        vg = v[:, :, idx_c, :].reshape(B, H, S, W, Dh)
        logits = jnp.einsum("bhsd,bhswd->bhsw", q, kg) * scale
        logits = jnp.where(mask[None, None, :, :], logits, -1e9)
        attn = _softmax(logits, axis=-1)
        o = jnp.einsum("bhsw,bhswd->bhsd", attn, vg)
        return (lambda x, *d: x.transpose(*d))(o, 0, 2, 1, 3).reshape(B, S, D) @ wo

    def _B_ref(x, wqkv, wo):
        B, S, D = x.shape
        H = 32; Dh = D // H
        W, dil = 8, 2
        qkv = (lambda x, *d: x.transpose(*d))((x @ wqkv).reshape(B, S, 3, H, Dh), 2, 0, 3, 1, 4)
        q, k, v = qkv[0], qkv[1], qkv[2]
        scale = Dh ** -0.5
        pos = jnp.arange(S)
        off = jnp.arange(W) * dil
        idx = pos[:, None] - off[None, :]
        mask = idx >= 0
        idx_c = jnp.where(mask, idx, 0).reshape(-1)
        kg = k[:, :, idx_c, :].reshape(B, H, S, W, Dh)
        vg = v[:, :, idx_c, :].reshape(B, H, S, W, Dh)
        logits = jnp.einsum("bhsd,bhswd->bhsw", q, kg) * scale
        logits = jnp.where(mask[None, None, :, :], logits, -1e9)
        attn = _softmax(logits, axis=-1)
        o = jnp.einsum("bhsw,bhswd->bhsd", attn, vg)
        return (lambda x, *d: x.transpose(*d))(o, 0, 2, 1, 3).reshape(B, S, D) @ wo

    x = A_x
    x = x + _A_ref(_layernorm(x, axis=-1), A_wqkv, A_wo)
    x = x + _B_ref(_layernorm(x, axis=-1), B_wqkv, B_wo)
    x = x + _A_ref(_layernorm(x, axis=-1), A_wqkv, A_wo)
    x = x + _B_ref(_layernorm(x, axis=-1), B_wqkv, B_wo)
    return x
```

```python
import math

import jax
import jax.numpy as jnp
from jax import lax
import jax.experimental.pallas as pl
import jax.experimental.pallas.tpu as pltpu

S, D, H, DH, WIN, DIL = 2048, 1024, 32, 32, 8, 2
NL = 4
LANES = 128
NC = D // LANES
HC = NC // 2
HD = D // 2
HALO = 16
def _f(n, k=0):
    return tuple(i for i in range(32) if (i + k + 1) * n // 32 > (i + k) * n // 32)


CFG = dict(TM=256, NCH=256, NCC=128, RG=32, LG=16, LOOPONLY=0, FLAGS={}, ONE=(0, 4, 7, 11, 15, 18, 22, 25, 29), ONEP=(24, 17, 17, 28), PR=32, WCH=4, MG=16, PB=1, INF=(2, 2), CH=32, QS=2, LS=0, WL=2, WD=0, CB=0, CH0=False, LF=1.0, CP=1.0, LO=0.0)


def _kernel(x_hbm, wqkv_a, wo_a, wqkv_b, wo_b, out_hbm,
            wqkv, wo, wqkv_raw, wo_raw, wo_tmp, pbuf, obuf, xin, xres0, xres1, ostage,
            xn0, xn1, q0, q1, k0, k1, v0, v1, o0, o1,
            flag, sem_x, sem_q, sem_w, sem_o):
    TM, NCH, NCC, RG, LG, WCH = (CFG[n] for n in ("TM", "NCH", "NCC", "RG", "LG", "WCH"))
    T = S // TM
    HM = TM // 2
    xn, qb, kb, vb, ob = (xn0, xn1), (q0, q1), (k0, k1), (v0, v1), (o0, o1)
    xres = (xres0, xres1)
    f32, bf16, i32 = jnp.float32, jnp.bfloat16, jnp.int32

    def pack(x):
        return pltpu.bitcast(x.astype(bf16), i32)

    def unpack(x):
        return pltpu.bitcast(x, bf16)

    flag[0] = 1

    def after(x, earlier, u=0):
        if earlier is None:
            return x
        return jnp.where(flag[0] > 0 if static(u) else u >= 0, x, earlier)

    def lanes(c, n=LANES):
        return pl.ds(c * LANES, n)

    def static(u):
        return isinstance(u, int)

    def tile(u):
        return u % T if static(u) else lax.rem(u, T)

    def half(t):
        return t // 2 if static(t) else lax.div(t, 2)

    def weight_set(u):
        return (u // T) % 2 if static(u) else lax.rem(lax.div(u, T), 2)

    def x_copy(t, n=1):
        r = pl.ds(t * TM, n * TM)
        return pltpu.make_async_copy(x_hbm.at[r], xin.at[r], sem_x.at[t])

    def first_copy(i):
        r, c = pl.ds(i * (D // WCH), D // WCH), pl.ds(0, D)
        return pltpu.make_async_copy(wqkv_a.at[r, c], wqkv_raw.at[0, r, c], sem_q.at[i])

    def wqkv_copy(s, p):
        c = pl.ds(p * D, D)
        return pltpu.make_async_copy((wqkv_a, wqkv_b)[s].at[:, c], wqkv_raw.at[s, :, c], sem_w.at[s * 4 + p])

    def wo_copy(s):
        return pltpu.make_async_copy((wo_a, wo_b)[s], wo_raw.at[s], sem_w.at[s * 4 + 3])

    def out_copy(t):
        r = pl.ds(t * TM if static(t) else pl.multiple_of(t * TM, TM), TM)
        return pltpu.make_async_copy(ostage.at[t], out_hbm.at[r], sem_o.at[t])

    def start(*copies):
        for c in copies:
            c.start()

    def wait(*copies):
        for c in copies:
            c.wait()

    def lhs_terms(a11, a12, a21, a22):
        return (a11 + a22, a21 + a22, a11, a22, a11 + a12, a21 - a11, a12 - a22)

    def rhs_terms(b11, b12, b21, b22):
        return (b11 + b22, b11, b12 - b22, b21 - b11, b22, b11 + b12, b21 + b22)

    def block_product(lhs, rhs, emit):
        def mm(i):
            return jnp.dot(lhs(i - 1), unpack(rhs(i - 1)), preferred_element_type=f32)

        m2 = mm(2)
        m4 = mm(4)
        emit(2, m2 + m4)
        c22 = mm(6) - m2
        m1 = mm(1)
        c11 = m1 + m4
        c22 = c22 + m1
        c11 = c11 + mm(7)
        m5 = mm(5)
        emit(0, c11 - m5)
        m3 = mm(3)
        emit(1, m3 + m5)
        emit(3, c22 + m3)

    def prep_wqkv(s, p, R=16):

        def piece(r0):
            def run():
                lane = lax.broadcasted_iota(i32, (R // 2, LANES), 1)
                halves = []
                for e in range(2):
                    row = (r0 // LANES * 2 + e) * LANES + r0 % LANES
                    t = [pltpu.bitcast(wqkv_raw[s, pl.ds(row, R), lanes(p * NC + a)], i32)
                         for a in range(NC)]
                    for st in (1, 2, 4):
                        keep = (lane & (4 * st)) == 0
                        for a in range(NC):
                            if a & st == 0:
                                lo, hi = t[a], t[a + st]
                                t[a] = jnp.where(keep, lo, hi)
                                t[a + st] = jnp.where(keep, hi, lo)
                    halves.append(t)
                top, bot = halves
                for c in range(NC):
                    src = (lane & 3) * 32 + ((lane & 28) ^ (4 * c)) + (lane >> 5)
                    top[c] = jnp.take_along_axis(top[c], src, axis=1)
                    bot[c] = jnp.take_along_axis(bot[c], src, axis=1)
                for c in range(HC):
                    words = (top[c], top[c + HC], bot[c], bot[c + HC])
                    terms = rhs_terms(*(unpack(w).astype(f32) for w in words))
                    for i, w in enumerate(terms):
                        w = words[0] if i == 1 else words[3] if i == 4 else pack(w)
                        wqkv[s, i, pl.ds(r0 // 2, R // 2), lanes(p * HC + c)] = w
            return run
        return [piece(r0) for r0 in range(0, HD, R)]

    def prep_wo(s):
        pitch = DH + 1

        prev = [None] * CFG["WL"]

        def piece(cc):
            def run():
                for j in range(2):
                    for h in range(H):
                        wo_tmp[j, pl.ds(h * pitch, DH), :] = (
                            wo_raw[s, pl.ds(h * DH, DH), lanes(cc + j * HC)].astype(f32))
                low = lax.broadcasted_iota(i32, (8, LANES), 0) < 4

                def rows(j, c, dl, h0):
                    out = []
                    for h in (h0, h0 + 8):
                        a, b = (wo_tmp[j, pl.ds(h * pitch + 4 * ((h // 4 + e) ^ c) + dl, 8, stride=pitch), :]
                                for e in range(2))
                        out.append(jnp.where(low, a, b))
                    return jnp.concatenate(out, axis=0)

                for c in range(HC):
                    for dl in range(4):
                        for h0 in (0, 16):
                            terms = rhs_terms(*(rows(j, c + e, dl, h0) for e in (0, HC) for j in range(2)))
                            for i, w in enumerate(terms):
                                w = pack(jnp.concatenate([after(w[:8], prev.pop(0)), w[8:]], axis=0))
                                wo[s, i, pl.ds((c * LANES + dl * H + h0) // 2, 8), lanes(cc)] = w
                                prev.append(pltpu.bitcast(w, f32))
            return run
        return [piece(cc) for cc in range(HC)]

    def widen_x(t):
        def run():
            prev = None
            for u in range(t, T):
                for r0 in range(0, TM, 16):
                    x = xin[pl.ds(u * TM + r0, 16), :].astype(f32)
                    if CFG["WD"]:
                        x = after(x, prev)
                    xres[u % 2][u // 2, pl.ds(r0, 16), :] = x
                    prev = x
        return [run]

    def stage_l(u, par):
        slot = half(tile(u))

        def norm(r0):
            r = pl.ds(r0, LG)
            if static(u):
                x = xin[pl.ds(u * TM + r0, LG), :].astype(f32)
                xres[par][slot, r, :] = x
            else:
                x = xres[par][slot, r, :]
            if not CFG["LS"]:
                xc = x - jnp.mean(x, axis=-1, keepdims=True)
                var = jnp.mean(xc * xc, axis=-1, keepdims=True)
                return xc * lax.rsqrt(var + 1e-5)
            xs = [x[:, c * LANES:(c + 1) * LANES] for c in range(NC)]
            tot = xs[0]
            for y in xs[1:]:
                tot = tot + y
            mean = jnp.broadcast_to(jnp.sum(tot, axis=-1, keepdims=True) * (1.0 / D), tot.shape)
            xcs, sq = [], None
            for y in xs:
                y = y - (after(mean, sq) if CFG["LS"] > 1 else mean)
                xcs.append(y)
                sq = y * y if sq is None else sq + y * y
            inv = lax.rsqrt(jnp.sum(sq, axis=-1, keepdims=True) * (1.0 / D) + 1e-5)
            return jnp.concatenate([y * inv for y in xcs], axis=1)

        def piece(r0):
            def run():
                top, bot = norm(r0), norm(HM + r0)
                blocks = [jnp.concatenate([y[:, c * LANES:(c + 1) * LANES] for c in range(e, NC, 2)], axis=1)
                          for y in (top, bot) for e in range(2)]
                for i, a in enumerate(lhs_terms(*blocks)):
                    xn[par][i, pl.ds(r0, LG), :] = a.astype(bf16)
            return run
        return [piece(r0) for r0 in range(0, HM, LG)]

    def stage_a(u, par):
        s = weight_set(u)

        def piece(n0):
            def run():
                dst, off = ((qb, 0), (kb, HALO), (vb, HALO))[n0 // HD]

                def emit(j, y):
                    for e in range(NCH // LANES):
                        c = (n0 % HD) // LANES + e + (j % 2) * HC
                        dst[par][c, pl.ds(off + (j // 2) * HM, HM), :] = y[:, e * LANES:(e + 1) * LANES]

                block_product(lambda i: xn[par][i], lambda i: wqkv[s, i, :, pl.ds(n0, NCH)], emit)
            return run
        return [piece(n0) for n0 in range(0, 3 * HD, NCH)]

    def stage_b(u, par, flat, chain=True):
        first = tile(u) == 0
        scale = DH ** -0.5
        q, k, v = qb[par], kb[par], vb[par]

        def probs(r0):
            qs = [q[c, pl.ds(r0, 8), :] for c in range(NC)]
            acc = []
            QS = CFG["QS"]
            for w in range(WIN):
                rows = pl.ds(HALO + r0 - DIL * w, 8)
                t = after(qs[0], acc[w - QS] if QS and chain and w >= QS else None, u) * k[0, rows, :]
                for c in range(1, NC):
                    t = t + qs[c] * k[c, rows, :]
                acc.append(t)
            lg = []
            for w in range(WIN):
                t = acc[w] + pltpu.roll(acc[w], 2 * H, 1)
                if (r0 // 8) in flat:
                    t = t + (pltpu.roll(acc[w], H, 1) + pltpu.roll(acc[w], 3 * H, 1))
                else:
                    t = t + pltpu.roll(t, H, 1)
                if r0 < DIL * w and first is not False:
                    pos = lax.broadcasted_iota(i32, (8, LANES), 0) + r0
                    t = jnp.where(jnp.logical_and(first, pos < DIL * w), -1e9 / scale, t)
                lg.append(t)
            m = lg[0]
            for w in range(1, WIN):
                m = jnp.maximum(m, lg[w])
            e = [jnp.exp2((t - m) * (scale * math.log2(math.e))) for t in lg]
            den = e[0]
            for w in range(1, WIN):
                den = den + e[w]
            inv = 1.0 / den
            for w in range(WIN):
                pbuf[w, pl.ds(r0, 8), :] = e[w] * inv

        def mix(r0, n):
            CH = CFG["CH"]
            prev = None
            for r in range(r0, r0 + n, CH):
                pr = [pbuf[w, pl.ds(r, CH), :] for w in range(WIN)]
                for c in range(NC):
                    o = after(pr[0], prev if chain else None, u) * v[c, pl.ds(HALO + r, CH), :]
                    for w in range(1, WIN):
                        o = o + pr[w] * v[c, pl.ds(HALO + r - DIL * w, CH), :]
                    obuf[pl.ds(r, CH), lanes(c)] = o
                    prev = o

        def fix_halo():
            for c in range(NC):
                for buf in (k, v):
                    row0 = jnp.broadcast_to(buf[c, pl.ds(HALO, 1), :], (HALO, LANES))
                    if first is True:
                        buf[c, pl.ds(0, HALO), :] = row0
                    elif first is not False:
                        buf[c, pl.ds(0, HALO), :] = jnp.where(first, row0, buf[c, pl.ds(0, HALO), :])

        def pass_halo():
            for c in range(NC):
                kb[1 - par][c, pl.ds(0, HALO), :] = k[c, pl.ds(TM, HALO), :]
                vb[1 - par][c, pl.ds(0, HALO), :] = v[c, pl.ds(TM, HALO), :]

        def piece(r0):
            def run():
                if r0 == 0:
                    fix_halo()
                for base in (r0, HM + r0):
                    for r in range(base, base + RG, 8):
                        probs(r)
                    mix(base, RG)
                CB = CFG["CB"] or RG
                prev = None
                for r in range(r0, r0 + RG, CB):
                    top, bot = pl.ds(r, CB), pl.ds(HM + r, CB)
                    for c in range(0, HC, 2):
                        left, right = lanes(c, 2 * LANES), lanes(c + HC, 2 * LANES)
                        a11, a22 = (after(y, prev) for y in (obuf[top, left], obuf[bot, right]))
                        terms = lhs_terms(a11, obuf[top, right], obuf[bot, left], a22)
                        for i, a in enumerate(terms):
                            ob[par][i, top, left] = a.astype(bf16)
                        if CFG["CB"] and chain:
                            prev = terms[-1]
                if r0 + RG == HM:
                    pass_halo()
            return run
        return [piece(r0) for r0 in range(0, HM, RG)]

    def stage_c(u, par):
        s = weight_set(u)
        t = tile(u)
        slot = half(t)

        def piece(n0):
            def run():
                def emit(j, y):
                    r, c = pl.ds((j // 2) * HM, HM), pl.ds((j % 2) * HD + n0, NCC)
                    xnew = xres[par][slot, r, c] + y
                    xres[par][slot, r, c] = xnew
                    ostage[t, r, c] = xnew.astype(bf16)

                block_product(lambda i: ob[par][i], lambda i: wo[s, i, :, pl.ds(n0, NCC)], emit)
            return run
        return [piece(n0) for n0 in range(0, HD, NCC)]

    def run(name, *stages):
        if CFG["LOOPONLY"] and name != "loop":
            return
        keyed = [((i + (CFG["LO"] if j == 1 else 0.5)) / len(st) * (CFG["LF"] if j == 1 else 1), j, f) for j, st in enumerate(stages) for i, f in enumerate(st)]
        for _, _, f in sorted(keyed, key=lambda item: item[:2]):
            f()

    def step(name, g, par, flat, *extra):
        sa, sc = stage_a(g, par), stage_c(g - 2, par)
        cut = int(len(sa) * CFG["CP"])
        run(name, sa[:cut] + sc + sa[cut:],
            stage_l(g + 1, 1 - par), stage_b(g - 1, 1 - par, flat), *extra)

    ONEP = CFG["ONEP"]
    queue = ([x_copy(0)] + [first_copy(i) for i in range(WCH)]
             + [x_copy(1), wqkv_copy(0, 1), wqkv_copy(0, 2), wo_copy(0), x_copy(2, 2), wqkv_copy(1, 0),
                x_copy(4), wqkv_copy(1, 1), x_copy(5, T - 5), wqkv_copy(1, 2), wo_copy(1)])
    depth = CFG["INF"]
    start(*queue[:depth[0]])
    state = [0, depth[0]]

    def arrive(n):
        wait(*queue[state[0]:state[0] + n])
        state[0] += n
        upto = min(len(queue), state[0] + (depth[0] if state[0] <= WCH else depth[1]))
        start(*queue[state[1]:upto])
        state[1] = max(state[1], upto)

    arrive(1)
    run("l0", stage_l(0, 0))
    prep_q = prep_wqkv(0, 0, 64)
    per = len(prep_q) // WCH
    for i in range(WCH):
        arrive(1)
        run("prep_q", prep_q[i * per:(i + 1) * per])
    a0, a1 = stage_a(0, 0), stage_a(1, 1)
    n = len(a0) // 3
    arrive(1)
    run("q0", a0[:n], stage_l(1, 1))
    arrive(1)
    run("q1", a1[:n], prep_wqkv(0, 1))
    arrive(1)
    run("k0", a0[n:2 * n], prep_wqkv(0, 2))
    arrive(1)
    run("v0", a0[2 * n:], prep_wo(0))
    arrive(1)
    run("kv1", a1[n:], stage_l(2, 0), stage_b(0, 0, _f(ONEP[0]), CFG['CH0']))
    arrive(1)
    step("s2", 2, 0, _f(ONEP[1]), prep_wqkv(1, 0))
    arrive(2)
    step("s3", 3, 1, _f(ONEP[1]), prep_wqkv(1, 1))
    arrive(2)
    step("s4", 4, 0, _f(ONEP[1]), prep_wqkv(1, 2), widen_x(7))
    arrive(1)
    step("s5", 5, 1, _f(ONEP[2]), prep_wo(1))
    assert state == [len(queue)] * 2

    def loop_body(g, carry):
        for par in range(2):
            @pl.when(lax.rem(g, 2) == par)
            def _():
                step("loop", g, par, CFG["ONE"])

        @pl.when(g - 2 >= (NL - 1) * T)
        def _():
            out_copy(tile(g - 2)).start()
        return carry

    last = NL * T - 1
    lax.fori_loop(6, last + 1, loop_body, None)

    run("e0", stage_c(last - 1, 0), stage_b(last, 1, _f(ONEP[3]), False))
    start(out_copy(T - 2))
    run("e1", stage_c(last, 1))
    start(out_copy(T - 1))
    wait(*(out_copy(t) for t in range(T)))


@jax.jit
def pallas_interleave_layers__sliding_local_dilated__sliding_local_dilated__prompt_kernel(
        A_x, A_wqkv, A_wo, B_x, B_wqkv, B_wo):
    del B_x
    TM = CFG["TM"]
    T = S // TM
    f32, bf16, i32 = jnp.float32, jnp.bfloat16, jnp.int32
    vm = pltpu.VMEM
    scratch = [
        vm((2, 7, HD // 2, 3 * HD), i32), vm((2, 7, HD // 2, HD), i32),
        vm((2, D, 3 * D), bf16), vm((2, D, D), bf16), vm((2, H * (DH + 1), LANES), f32),
        vm((WIN, TM, LANES), f32), vm((TM, D), f32),
        vm((S, D), bf16), vm((T // 2, TM, D), f32), vm((T // 2, TM, D), f32), vm((T, TM, D), bf16),
        vm((7, TM // 2, HD), bf16), vm((7, TM // 2, HD), bf16),
        vm((NC, TM, LANES), f32), vm((NC, TM, LANES), f32),
        vm((NC, HALO + TM, LANES), f32), vm((NC, HALO + TM, LANES), f32),
        vm((NC, HALO + TM, LANES), f32), vm((NC, HALO + TM, LANES), f32),
        vm((7, TM // 2, HD), bf16), vm((7, TM // 2, HD), bf16),
        pltpu.SMEM((1,), i32),
        pltpu.SemaphoreType.DMA((T,)), pltpu.SemaphoreType.DMA((CFG["WCH"],)),
        pltpu.SemaphoreType.DMA((8,)), pltpu.SemaphoreType.DMA((T,)),
    ]
    hbm = pl.BlockSpec(memory_space=pl.ANY)
    out = pl.pallas_call(
        _kernel,
        out_shape=jax.ShapeDtypeStruct((S, D), bf16),
        in_specs=[hbm] * 5,
        out_specs=hbm,
        scratch_shapes=scratch,
        compiler_params=pltpu.CompilerParams(vmem_limit_bytes=100 * 1024 * 1024, flags=CFG["FLAGS"] or None),
        name="fused_layers",
    )(A_x.reshape(S, D), A_wqkv, A_wo, B_wqkv, B_wo)
    return out.reshape(1, S, D)
```

```python
import math

import jax
import jax.numpy as jnp
import numpy as np
from jax import lax
import jax.experimental.pallas as pl
import jax.experimental.pallas.tpu as pltpu

S, D, H, DH, WIN, DIL = 2048, 1024, 32, 32, 8, 2
NL = 4
LANES = 128
NC = D // LANES
HC = NC // 2
HD = D // 2
HALO = 16
TM = 256
T = S // TM
HM = TM // 2
RG = 32
LG = 16
SP = 96

STEADY = ((0, 1, 3, 7, 11, 15, 19, 22, 25, 30), 128, 0.75, True)
WARM_UP = (
    ((1, 3, 5, 7, 9, 10, 13, 14, 16, 18, 20, 22, 24, 26, 28, 30, 31), 128, 0.0, False),
    ((1, 3, 5, 7, 9, 10, 11, 13, 14, 16, 18, 20, 22, 24, 26, 28, 30, 31), 128, 0.0, False),
    ((1, 3, 5, 7, 9, 11, 13, 16, 18, 20, 21, 24, 26, 28, 30, 31), 256, 0.0, False),
    ((0, 1, 3, 5, 6, 9, 12, 13, 15, 16, 18, 20, 21, 22, 24, 26, 28, 30), 256, 0.0, False),
)
FIRST_FLAT = (0, 2, 4, 5, 6, 7, 9, 10, 11, 12, 13, 15, 17, 18, 20, 21, 22, 23, 25, 26, 27, 28, 29, 31)
LAST_FLAT = tuple(i for i in range(TM // 8) if i % 8)


def _kernel(one, x_hbm, wqkv_a, wo_a, wqkv_b, wo_b, out_hbm,
            wqkv, wo, wqkv_raw, wo_raw, wo_tmp, pbuf, obuf, xin, xres0, xres1, ostage,
            xn0, xn1, q0, q1, k0, k1, v0, v1, o0, o1,
            sem_x, sem_q, sem_w, sem_o):
    xn, qb, kb, vb, ob = (xn0, xn1), (q0, q1), (k0, k1), (v0, v1), (o0, o1)
    xres = (xres0, xres1)
    f32, bf16, i32 = jnp.float32, jnp.bfloat16, jnp.int32

    def pack(x):
        return pltpu.bitcast(x.astype(bf16), i32)

    def unpack(x):
        return pltpu.bitcast(x, bf16)

    def after(x, earlier, u=0):
        if earlier is None:
            return x
        return jnp.where(one[0] > 0 if static(u) else u >= 0, x, earlier)

    def lanes(c, n=LANES):
        return pl.ds(c * LANES, n)

    def static(u):
        return isinstance(u, int)

    def tile(u):
        return u & (T - 1)

    def half(t):
        return t >> 1

    def weight_set(u):
        return (u >> (T.bit_length() - 1)) & 1

    def x_copy(t, n=1):
        r = pl.ds(t * TM, n * TM)
        return pltpu.make_async_copy(x_hbm.at[r], xin.at[r], sem_x.at[t])

    def first_copy(i):
        r, c = pl.ds(i * HD, HD), pl.ds(0, D)
        return pltpu.make_async_copy(wqkv_a.at[r, c], wqkv_raw.at[0, r, c], sem_q.at[i])

    def wqkv_copy(s, p):
        c = pl.ds(p * D, D)
        return pltpu.make_async_copy((wqkv_a, wqkv_b)[s].at[:, c], wqkv_raw.at[s, :, c], sem_w.at[s * 4 + p])

    def wo_copy(s):
        return pltpu.make_async_copy((wo_a, wo_b)[s], wo_raw.at[s], sem_w.at[s * 4 + 3])

    def out_copy(t):
        r = pl.ds(t * TM if static(t) else pl.multiple_of(t * TM, TM), TM)
        return pltpu.make_async_copy(ostage.at[t], out_hbm.at[r], sem_o.at[t])

    def start(*copies):
        for c in copies:
            c.start()

    def wait(*copies):
        for c in copies:
            c.wait()

    def lhs_terms(a11, a12, a21, a22):
        return (a11 + a22, a21 + a22, a11, a22, a11 + a12, a21 - a11, a12 - a22)

    def rhs_terms(b11, b12, b21, b22):
        return (b11 + b22, b11, b12 - b22, b21 - b11, b22, b11 + b12, b21 + b22)

    def block_product(lhs, rhs, emit):
        def mm(i):
            return jnp.dot(lhs(i - 1), unpack(rhs(i - 1)), preferred_element_type=f32)

        m2 = mm(2)
        m4 = mm(4)
        emit(2, m2 + m4)
        c22 = mm(6) - m2
        m1 = mm(1)
        c11 = m1 + m4
        c22 = c22 + m1
        c11 = c11 + mm(7)
        m5 = mm(5)
        emit(0, c11 - m5)
        m3 = mm(3)
        emit(1, m3 + m5)
        emit(3, c22 + m3)

    def prep_wqkv(s, p, R=16):

        def piece(r0):
            def run():
                lane = lax.broadcasted_iota(i32, (R // 2, LANES), 1)
                halves = []
                for e in range(2):
                    row = (r0 // LANES * 2 + e) * LANES + r0 % LANES
                    t = [pltpu.bitcast(wqkv_raw[s, pl.ds(row, R), lanes(p * NC + a)], i32)
                         for a in range(NC)]
                    for st in (1, 2, 4):
                        keep = (lane & (4 * st)) == 0
                        for a in range(NC):
                            if a & st == 0:
                                lo, hi = t[a], t[a + st]
                                t[a] = jnp.where(keep, lo, hi)
                                t[a + st] = jnp.where(keep, hi, lo)
                    halves.append(t)
                top, bot = halves
                for c in range(NC):
                    src = (lane & 3) * 32 + ((lane & 28) ^ (4 * c)) + (lane >> 5)
                    top[c] = jnp.take_along_axis(top[c], src, axis=1)
                    bot[c] = jnp.take_along_axis(bot[c], src, axis=1)
                for c in range(HC):
                    words = (top[c], top[c + HC], bot[c], bot[c + HC])
                    terms = rhs_terms(*(unpack(w).astype(f32) for w in words))
                    for i, w in enumerate(terms):
                        w = words[0] if i == 1 else words[3] if i == 4 else pack(w)
                        wqkv[s, i, pl.ds(r0 // 2, R // 2), lanes(p * HC + c)] = w
            return run
        return [piece(r0) for r0 in range(0, HD, R)]

    def prep_wo(s):
        pitch = DH + 1

        prev = [None, None]

        def piece(cc):
            def run():
                for j in range(2):
                    for h in range(H):
                        wo_tmp[j, pl.ds(h * pitch, DH), :] = (
                            wo_raw[s, pl.ds(h * DH, DH), lanes(cc + j * HC)].astype(f32))
                low = lax.broadcasted_iota(i32, (8, LANES), 0) < 4

                def rows(j, c, dl, h0):
                    out = []
                    for h in (h0, h0 + 8):
                        a, b = (wo_tmp[j, pl.ds(h * pitch + 4 * ((h // 4 + e) ^ c) + dl, 8, stride=pitch), :]
                                for e in range(2))
                        out.append(jnp.where(low, a, b))
                    return jnp.concatenate(out, axis=0)

                for c in range(HC):
                    for dl in range(4):
                        for h0 in (0, 16):
                            terms = rhs_terms(*(rows(j, c + e, dl, h0) for e in (0, HC) for j in range(2)))
                            for i, w in enumerate(terms):
                                w = pack(jnp.concatenate([after(w[:8], prev.pop(0)), w[8:]], axis=0))
                                wo[s, i, pl.ds((c * LANES + dl * H + h0) // 2, 8), lanes(cc)] = w
                                prev.append(pltpu.bitcast(w, f32))
            return run
        return [piece(cc) for cc in range(HC)]

    def widen_x(t):
        def run():
            xres[t % 2][t // 2] = xin[pl.ds(t * TM, TM), :].astype(f32)
        return [run]

    def stage_l(u, par, chain=False):
        slot = half(tile(u))

        def norm(r0):
            r = pl.ds(r0, LG)
            if static(u):
                x = xin[pl.ds(u * TM + r0, LG), :].astype(f32)
                xres[par][slot, r, :] = x
            else:
                x = xres[par][slot, r, :]
            if not chain:
                xc = x - jnp.mean(x, axis=-1, keepdims=True)
                var = jnp.mean(xc * xc, axis=-1, keepdims=True)
                return xc * lax.rsqrt(var + 1e-5)
            xs = [x[:, c * LANES:(c + 1) * LANES] for c in range(NC)]
            tot = xs[0]
            for y in xs[1:]:
                tot = tot + y
            mean = jnp.broadcast_to(jnp.sum(tot, axis=-1, keepdims=True) * (1.0 / D), tot.shape)
            xcs, sq = [], None
            for y in xs:
                y = y - after(mean, sq)
                xcs.append(y)
                sq = y * y if sq is None else sq + y * y
            inv = lax.rsqrt(jnp.sum(sq, axis=-1, keepdims=True) * (1.0 / D) + 1e-5)
            return jnp.concatenate([y * inv for y in xcs], axis=1)

        def piece(r0):
            def run():
                top, bot = norm(r0), norm(HM + r0)
                blocks = [jnp.concatenate([y[:, c * LANES:(c + 1) * LANES] for c in range(e, NC, 2)], axis=1)
                          for y in (top, bot) for e in range(2)]
                for i, a in enumerate(lhs_terms(*blocks)):
                    xn[par][i, pl.ds(r0, LG), :] = a.astype(bf16)
            return run
        return [piece(r0) for r0 in range(0, HM, LG)]

    def stage_a(u, par, width):
        s = weight_set(u)

        def piece(n0):
            def run():
                dst, off = ((qb, 0), (kb, HALO), (vb, HALO))[n0 // HD]

                def emit(j, y):
                    for e in range(width // LANES):
                        c = (n0 % HD) // LANES + e + (j % 2) * HC
                        dst[par][c, pl.ds(off + (j // 2) * HM, HM), :] = y[:, e * LANES:(e + 1) * LANES]

                block_product(lambda i: xn[par][i], lambda i: wqkv[s, i, :, pl.ds(n0, width)], emit)
            return run
        return [piece(n0) for n0 in range(0, 3 * HD, width)]

    def stage_b(u, par, flat, chain=2):
        first = tile(u) == 0
        scale = DH ** -0.5
        q, k, v = qb[par], kb[par], vb[par]

        def probs(r0):
            qs = [q[c, pl.ds(r0, 8), :] for c in range(NC)]
            acc = []
            for w in range(WIN):
                rows = pl.ds(HALO + r0 - DIL * w, 8)
                t = after(qs[0], acc[w - 2] if chain > 1 and w >= 2 else None, u) * k[0, rows, :]
                for c in range(1, NC):
                    t = t + qs[c] * k[c, rows, :]
                acc.append(t)
            lg = []
            for w in range(WIN):
                t = acc[w] + pltpu.roll(acc[w], 2 * H, 1)
                if (r0 // 8) in flat:
                    t = t + (pltpu.roll(acc[w], H, 1) + pltpu.roll(acc[w], 3 * H, 1))
                else:
                    t = t + pltpu.roll(t, H, 1)
                if r0 < DIL * w and first is not False:
                    pos = lax.broadcasted_iota(i32, (8, LANES), 0) + r0
                    t = jnp.where(jnp.logical_and(first, pos < DIL * w), -1e9 / scale, t)
                lg.append(t)
            m = lg[0]
            for w in range(1, WIN):
                m = jnp.maximum(m, lg[w])
            e = [jnp.exp2((t - m) * (scale * math.log2(math.e))) for t in lg]
            den = e[0]
            for w in range(1, WIN):
                den = den + e[w]
            inv = 1.0 / den
            for w in range(WIN):
                pbuf[w, pl.ds(r0, 8), :] = e[w] * inv

        def mix(r0):
            pr = [pbuf[w, pl.ds(r0, RG), :] for w in range(WIN)]
            o = None
            for c in range(NC):
                o = after(pr[0], o if chain else None, u) * v[c, pl.ds(HALO + r0, RG), :]
                for w in range(1, WIN):
                    o = o + pr[w] * v[c, pl.ds(HALO + r0 - DIL * w, RG), :]
                obuf[pl.ds(r0, RG), lanes(c)] = o

        def fix_halo():
            for c in range(NC):
                for buf in (k, v):
                    row0 = jnp.broadcast_to(buf[c, pl.ds(HALO, 1), :], (HALO, LANES))
                    if first is True:
                        buf[c, pl.ds(0, HALO), :] = row0
                    elif first is not False:
                        buf[c, pl.ds(0, HALO), :] = jnp.where(first, row0, buf[c, pl.ds(0, HALO), :])

        def pass_halo():
            for c in range(NC):
                kb[1 - par][c, pl.ds(0, HALO), :] = k[c, pl.ds(TM, HALO), :]
                vb[1 - par][c, pl.ds(0, HALO), :] = v[c, pl.ds(TM, HALO), :]

        def piece(r0):
            def run():
                if r0 == 0:
                    fix_halo()
                for base in (r0, HM + r0):
                    for r in range(base, base + RG, 8):
                        probs(r)
                    mix(base)
                top, bot = pl.ds(r0, RG), pl.ds(HM + r0, RG)
                for c in range(0, HC, 2):
                    left, right = lanes(c, 2 * LANES), lanes(c + HC, 2 * LANES)
                    a11, a22 = obuf[top, left], obuf[bot, right]
                    for i, a in enumerate(lhs_terms(a11, obuf[top, right], obuf[bot, left], a22)):
                        ob[par][i, top, left] = a.astype(bf16)
                if r0 + RG == HM:
                    pass_halo()
            return run
        return [piece(r0) for r0 in range(0, HM, RG)]

    def stage_c(u, par, r0=0, n=HM):
        s = weight_set(u)
        t = tile(u)
        slot = half(t)

        def piece(n0):
            def run():
                def emit(j, y):
                    r, c = pl.ds((j // 2) * HM + r0, n), pl.ds((j % 2) * HD + n0, LANES)
                    xnew = xres[par][slot, r, c] + y
                    xres[par][slot, r, c] = xnew
                    ostage[t, r, c] = xnew.astype(bf16)

                block_product(lambda i: ob[par][i, pl.ds(r0, n), :], lambda i: wo[s, i, :, pl.ds(n0, LANES)], emit)
            return run
        return [piece(n0) for n0 in range(0, HD, LANES)]

    def run(*stages, lo=0.5):
        keyed = [((i + (lo if j == 1 else 0.5)) / len(st), j, f) for j, st in enumerate(stages) for i, f in enumerate(st)]
        for _, _, f in sorted(keyed, key=lambda item: item[:2]):
            f()

    def step(g, par, tune, *extra):
        flat, width, lo, chain = tune
        run(stage_a(g, par, width) + stage_c(g - 2, par),
            stage_l(g + 1, 1 - par, chain), stage_b(g - 1, 1 - par, flat), *extra, lo=lo)

    start(x_copy(0), first_copy(0))
    wait(x_copy(0))
    start(first_copy(1))
    run(stage_l(0, 0))
    prep_q = prep_wqkv(0, 0, 64)
    per = len(prep_q) // 2
    for i, then in enumerate((x_copy(1), wqkv_copy(0, 1))):
        wait(first_copy(i))
        start(then)
        run(prep_q[i * per:(i + 1) * per])
    a0, a1 = stage_a(0, 0, LANES), stage_a(1, 1, LANES)
    n = len(a0) // 3
    wait(x_copy(1))
    start(wqkv_copy(0, 2))
    run(a0[:n], stage_l(1, 1))
    wait(wqkv_copy(0, 1))
    start(wo_copy(0))
    run(a1[:n], prep_wqkv(0, 1))
    wait(wqkv_copy(0, 2))
    start(x_copy(2, 2))
    run(a0[n:2 * n], prep_wqkv(0, 2))
    wait(wo_copy(0))
    start(wqkv_copy(1, 0))
    run(a0[2 * n:], prep_wo(0))
    wait(x_copy(2, 2))
    start(wqkv_copy(1, 1))
    run(a1[n:], stage_l(2, 0), stage_b(0, 0, FIRST_FLAT, 1), lo=0.0)
    wait(wqkv_copy(1, 0), wqkv_copy(1, 1))
    start(x_copy(4, T - 4), wo_copy(1))
    step(2, 0, WARM_UP[0], prep_wqkv(1, 0))
    wait(x_copy(4, T - 4))
    start(wqkv_copy(1, 2))
    step(3, 1, WARM_UP[1], prep_wqkv(1, 1))
    wait(wo_copy(1))
    step(4, 0, WARM_UP[2], prep_wo(1))
    wait(wqkv_copy(1, 2))
    step(5, 1, WARM_UP[3], prep_wqkv(1, 2), widen_x(7))

    def loop_body(g, carry):
        for par in range(2):
            @pl.when(g & 1 == par)
            def _():
                step(g, par, STEADY)

        @pl.when(g - 2 >= (NL - 1) * T)
        def _():
            out_copy(tile(g - 2)).start()
        return carry

    last = NL * T - 1
    lax.fori_loop(6, last + 1, loop_body, None)

    def tail_copies(i):
        rows = [pl.ds(base + i * SP, HM - SP if i else SP) for base in (0, HM)]
        return [pltpu.make_async_copy(ostage.at[T - 1, r], out_hbm.at[pl.ds((T - 1) * TM + r.start, r.size)],
                                      sem_o.at[T - 1 + 2 * i + j]) for j, r in enumerate(rows)]

    run(stage_c(last - 1, 0), stage_b(last, 1, LAST_FLAT, 0))
    start(out_copy(T - 2))
    run(stage_c(last, 1, 0, SP))
    start(*tail_copies(0))
    run(stage_c(last, 1, SP, HM - SP))
    start(*tail_copies(1))
    wait(*(out_copy(t) for t in range(T - 1)), *tail_copies(0), *tail_copies(1))


@jax.jit
def pallas_interleave_layers__sliding_local_dilated__sliding_local_dilated__prompt_kernel(
        A_x, A_wqkv, A_wo, B_x, B_wqkv, B_wo):
    del B_x
    f32, bf16, i32 = jnp.float32, jnp.bfloat16, jnp.int32
    vm = pltpu.VMEM
    scratch = [
        vm((2, 7, HD // 2, 3 * HD), i32), vm((2, 7, HD // 2, HD), i32),
        vm((2, D, 3 * D), bf16), vm((2, D, D), bf16), vm((2, (H + 2) * (DH + 1) // 8 * 8, LANES), f32),
        vm((WIN, TM, LANES), f32), vm((TM, D), f32),
        vm((S, D), bf16), vm((T // 2, TM, D), f32), vm((T // 2, TM, D), f32), vm((T, TM, D), bf16),
        vm((7, TM // 2, HD), bf16), vm((7, TM // 2, HD), bf16),
        vm((NC, TM, LANES), f32), vm((NC, TM, LANES), f32),
        vm((NC, HALO + TM, LANES), f32), vm((NC, HALO + TM, LANES), f32),
        vm((NC, HALO + TM, LANES), f32), vm((NC, HALO + TM, LANES), f32),
        vm((7, TM // 2, HD), bf16), vm((7, TM // 2, HD), bf16),
        pltpu.SemaphoreType.DMA((T,)), pltpu.SemaphoreType.DMA((2,)),
        pltpu.SemaphoreType.DMA((8,)), pltpu.SemaphoreType.DMA((T + 3,)),
    ]
    hbm = pl.BlockSpec(memory_space=pl.ANY)
    out = pl.pallas_call(
        _kernel,
        out_shape=jax.ShapeDtypeStruct((S, D), bf16),
        in_specs=[pl.BlockSpec(memory_space=pltpu.SMEM)] + [hbm] * 5,
        out_specs=hbm,
        scratch_shapes=scratch,
        compiler_params=pltpu.CompilerParams(vmem_limit_bytes=100 * 1024 * 1024),
        name="fused_layers",
    )(np.ones((1,), np.int32), A_x.reshape(S, D), A_wqkv, A_wo, B_wqkv, B_wo)
    return out.reshape(1, S, D)
```
